```python
import os as _os
_os.environ.setdefault("JAX_PLATFORMS", "cpu")
import jax
import jax.numpy as jnp

def _softmax(x, axis=-1):
    return jax.nn.softmax(x, axis=axis)
def _gelu(x):
    return jax.nn.gelu(x, approximate=True)
def _silu(x):
    return jax.nn.silu(x)
def _sigmoid(x):
    return jax.nn.sigmoid(x)
def _layernorm(x, axis=-1, eps=1e-5):
    m = jnp.mean(x, axis=axis, keepdims=True)
    v = jnp.var(x, axis=axis, keepdims=True)
    return (x - m) / jnp.sqrt(v + eps)
def _scatter_add(tgt, idx, src, axis=0):
    return tgt.at[idx].add(src)
def _segment_sum(src, seg, n):
    return jax.ops.segment_sum(src, seg, n)
class _Rng:
    def __init__(self, key):
        self._k = key
    def _next(self):
        self._k, sub = jax.random.split(self._k)
        return sub
    def normal(self, shape):
        return jax.random.normal(self._next(), shape, dtype=jnp.bfloat16)
    def randint(self, lo, hi, shape):
        return jax.random.randint(self._next(), shape, lo, hi, dtype=jnp.int32)
    def uniform(self, shape, lo=0.0, hi=1.0):
        return jax.random.uniform(self._next(), shape, jnp.bfloat16, lo, hi)
    def permutation(self, n):
        return jax.random.permutation(self._next(), n)


kernel_name = 'recurrent_scan__ssm_conv_s4__mixer_s_mlp__prompt'

def setup_inputs():
    _rng = _Rng(jax.random.key(int.from_bytes(__import__("os").urandom(4), "little")))
    _w = (lambda a: (lambda t: t.astype(jnp.bfloat16) if jnp.issubdtype(t.dtype, jnp.floating) else t)(jnp.asarray(a)))
    def _A_setup():
        B, L, D, N = 1, 2048, 512, 128
        A_re = -jnp.exp((lambda *s: _rng.normal(s) * 0.1)(D, N))
        A_im = jnp.pi * (lambda *s: _rng.normal(s) * 0.1)(D, N)
        B_re = (lambda *s: _rng.normal(s) * 0.1)(D, N)
        B_im = (lambda *s: _rng.normal(s) * 0.1)(D, N)
        C_re = (lambda *s: _rng.normal(s) * 0.1)(D, N)
        C_im = (lambda *s: _rng.normal(s) * 0.1)(D, N)
        log_dt = (lambda *s: _rng.normal(s) * 0.1)(D) * 0.5 - 4.0
        Dskip = (lambda *s: _rng.normal(s) * 0.05)(D)
        return {
            "u": _w((lambda *s: _rng.normal(s) * 0.05)(B, L, D)),
            "A_re": _w(A_re),
            "A_im": _w(A_im),
            "B_re": _w(B_re),
            "B_im": _w(B_im),
            "C_re": _w(C_re),
            "C_im": _w(C_im),
            "log_dt": _w(log_dt),
            "Dskip": _w(Dskip),
        }
    _A_in = _A_setup()

    def _B_setup():
        B, S, D, F = 1, 2048, 512, 1376
        return {
            "x":  _w((lambda *s: _rng.normal(s) * 0.05)(B, S, D)),
            "w1": _w((lambda *s: _rng.normal(s) * 0.8)(D, D) * (D ** -0.5)),
            "w2": _w((lambda *s: _rng.normal(s) * 0.8)(D, D) * (D ** -0.5)),
            "w3": _w((lambda *s: _rng.normal(s) * 0.8)(D, F) * (D ** -0.5)),
            "w4": _w((lambda *s: _rng.normal(s) * 0.8)(F, D) * (F ** -0.5)),
        }
    _B_in = _B_setup()

    return {
        "A_u": _A_in["u"],
        "A_A_re": _A_in["A_re"],
        "A_A_im": _A_in["A_im"],
        "A_B_re": _A_in["B_re"],
        "A_B_im": _A_in["B_im"],
        "A_C_re": _A_in["C_re"],
        "A_C_im": _A_in["C_im"],
        "A_log_dt": _A_in["log_dt"],
        "A_Dskip": _A_in["Dskip"],
        "B_x": _B_in["x"],
        "B_w1": _B_in["w1"],
        "B_w2": _B_in["w2"],
        "B_w3": _B_in["w3"],
        "B_w4": _B_in["w4"],
    }

def reference(A_u, A_A_re, A_A_im, A_B_re, A_B_im, A_C_re, A_C_im, A_log_dt, A_Dskip, B_x, B_w1, B_w2, B_w3, B_w4):
    def _A_ref(u, A_re, A_im, B_re, B_im, C_re, C_im, log_dt, Dskip):
        Bsz, L, D = u.shape
        dt = jnp.exp(log_dt)[:, None]
        A = A_re + 1j * A_im
        Bc = B_re + 1j * B_im
        Cc = C_re + 1j * C_im
        logdA = dt * A
        dB = dt * Bc
        l = (lambda x, dt: x.astype(dt))(jnp.arange(L), A_re.dtype)
        P = jnp.exp(logdA[:, :, None] * l[None, None, :])
        K = jnp.einsum("dn,dnl,dn->dl", Cc, P, dB).real
        L2 = 2 * L
        Kp = jnp.pad(K, ((0, 0), (0, L)))
        up = (lambda x, *d: x.transpose(*d))(u, 0, 2, 1)
        up = jnp.pad(up, ((0, 0), (0, 0), (0, L)))
        Kf = (lambda x, axes=(-2,-1): jnp.fft.rfft2(x.astype(jnp.float32), axes=axes))(Kp[:, None, :], axes=(-2, -1))
        Uf = (lambda x, axes=(-2,-1): jnp.fft.rfft2(x.astype(jnp.float32), axes=axes))(up[:, :, None, :], axes=(-2, -1))
        Yf = Uf * Kf[None, :, :, :]
        y = (lambda x, s, axes=(-2,-1): jnp.fft.irfft2(x, s=s, axes=axes).astype(jnp.bfloat16))(Yf, (1, L2), axes=(-2, -1))[:, :, 0, :L]
        y = (lambda x, *d: x.transpose(*d))(y, 0, 2, 1) + u * Dskip[None, None, :]
        return y

    def _B_ref(x, w1, w2, w3, w4):
        B, S, D = x.shape
        h = _gelu(_layernorm(x, axis=-1) @ w1)
        c = D // 4
        g0 = jnp.pad(h[:, :, 0*c:1*c], ((0, 0), (1, 0), (0, 0)))[:, :S, :]
        g1 = jnp.pad(h[:, :, 1*c:2*c], ((0, 0), (0, 1), (0, 0)))[:, 1:, :]
        g2 = jnp.pad(h[:, :, 2*c:3*c], ((0, 0), (2, 0), (0, 0)))[:, :S, :]
        g3 = jnp.pad(h[:, :, 3*c:   ], ((0, 0), (0, 2), (0, 0)))[:, 2:, :]
        hs = jnp.concatenate([g0, g1, g2, g3], axis=-1) @ w2
        x1 = x + hs
        h2 = _gelu(_layernorm(x1, axis=-1) @ w3) @ w4
        return x1 + h2

    x = A_u
    xn = _layernorm(x, axis=-1)
    s = _A_ref(xn, A_A_re, A_A_im, A_B_re, A_B_im, A_C_re, A_C_im, A_log_dt, A_Dskip)
    g = _silu(_B_ref(xn, B_w1, B_w2, B_w3, B_w4))
    return x + s * g
```

```python
import jax
import jax.numpy as jnp
import ml_dtypes
import numpy as np
import jax.experimental.pallas as pl
import jax.experimental.pallas.tpu as pltpu

L = 2048
D = 512
NS = 128
FF = 1376
R = 64
NFFT = R * R
NK1 = R // 2 + 1
TM = 256
HC = 256
PAD = 16
GC = 8
NG = D // GC
J = 16
BASES = (list(range(16)) + [256 + 2 * m for m in range(8)]
         + [512 + 4 * m for m in range(4)] + [768 + 4 * m for m in range(4)]
         + [1024 + 256 * q + 8 * m for q in range(4) for m in range(2)] + [2048])
NI = len(BASES)
KGROUPS = ([8, 16, 24, 4, 12, 20, 28, 0, 32],
           [1, 9, 17, 25, 7, 15, 23, 31],
           [2, 10, 18, 26, 6, 14, 22, 30],
           [3, 11, 19, 27, 5, 13, 21, 29])
KORD = [k for g in KGROUPS for k in g]
SLOT0 = [0, 9, 17, 25, 33]
RANGES = ((0, 256, 0), (256, 512, 2), (512, 1024, 3), (1024, 2048, 4))
NH = 6


def _lag_table():
    return np.arange(L).astype(ml_dtypes.bfloat16).astype(np.int64)


def _constants():
    bf = ml_dtypes.bfloat16
    t2 = np.arange(R)[None, :]
    k2 = np.arange(R)[:, None]
    m2 = np.zeros((NK1, 2 * R, 2 * R))
    for s, k1 in enumerate(KORD):
        th = -2 * np.pi * ((t2 * (k1 + R * k2)) % NFFT) / NFFT
        cr, ci = np.cos(th), np.sin(th)
        m2[s, :R, :R] = cr
        m2[s, :R, R:] = -ci
        m2[s, R:, :R] = ci
        m2[s, R:, R:] = cr
    m2i = np.transpose(m2, (0, 2, 1)) / NFFT
    lag = _lag_table()
    pos = {b + 16 * j: (i // 8) * 128 + (8 * j - i % 8) % 128 for i, b in enumerate(BASES) for j in range(J)}
    ex = np.zeros((L, 256))
    for start, stop, h0 in RANGES:
        for l in range(start, stop):
            ex[l, pos[int(lag[l])] - 128 * h0] = 1.0
    eye = np.concatenate([np.eye(128), np.kron(np.eye(16), np.eye(8)[::-1])], axis=0)
    return [c.astype(bf) for c in (
        m2.reshape(NK1 * 2 * R, 2 * R), m2i.reshape(NK1 * 2 * R, 2 * R), ex, eye)]


def _layernorm(x):
    m = jnp.mean(x, axis=-1, keepdims=True)
    xc = x - m
    v = jnp.mean(xc * xc, axis=-1, keepdims=True)
    return xc * lax_rsqrt(v + 1e-5)


def lax_rsqrt(v):
    return jax.lax.rsqrt(v)


def _gelu(x):
    c = np.float32(np.sqrt(2.0 / np.pi))
    return 0.5 * x * (1.0 + jnp.tanh(c * (x + 0.044715 * (x * x * x))))


def _cmul(ar, ai, br, bi):
    return ar * br - ai * bi, ar * bi + ai * br


def _cexp(er, ei):
    f = np.float32
    k = jnp.round(ei * f(1.0 / (2.0 * np.pi)))
    r = ((ei - k * f(6.28125)) - k * f(1.9350051879882812e-3)) - k * f(3.0199159819570e-7)
    y = 0.5 * r
    y2 = y * y
    sn = f(-1.0 / 39916800.0)
    for c in (1.0 / 362880.0, -1.0 / 5040.0, 1.0 / 120.0, -1.0 / 6.0, 1.0):
        sn = sn * y2 + f(c)
    sn = sn * y
    cs = f(-1.0 / 87178291200.0)
    for c in (1.0 / 479001600.0, -1.0 / 3628800.0, 1.0 / 40320.0, -1.0 / 720.0, 1.0 / 24.0, -0.5, 1.0):
        cs = cs * y2 + f(c)
    e = jnp.exp(er)
    e2 = e + e
    return e - e2 * (sn * sn), e2 * (sn * cs)


def _bdot(a, b):
    return jnp.dot(a, b, preferred_element_type=jnp.float32)


def _add(a, b):
    return b if a is None else (a if b is None else a + b)


def _sub(a, b):
    return a if b is None else (-b if a is None else a - b)


def _scale(a, c):
    if a is None or c == 0.0:
        return None
    return a if c == 1.0 else (-a if c == -1.0 else np.float32(c) * a)


def _cadd(a, b):
    return _add(a[0], b[0]), _add(a[1], b[1])


def _csub(a, b):
    return _sub(a[0], b[0]), _sub(a[1], b[1])


def _cconst(a, ang):
    ang %= 64
    cr, ci = np.cos(np.pi * ang / 32), np.sin(np.pi * ang / 32)
    if ang % 16 == 0:
        cr, ci = float(round(cr)), float(round(ci))
    return (_sub(_scale(a[0], cr), _scale(a[1], ci)), _add(_scale(a[0], ci), _scale(a[1], cr)))


def _dft8(a, sign):
    s = [_cadd(a[j], a[j + 4]) for j in range(4)]
    d = [_csub(a[j], a[j + 4]) for j in range(4)]
    e = [_cconst(d[j], sign * 8 * j) for j in range(4)]
    out = [None] * 8
    for off, v in ((0, s), (1, e)):
        p, m = _cadd(v[0], v[2]), _csub(v[0], v[2])
        q, r = _cadd(v[1], v[3]), _cconst(_csub(v[1], v[3]), sign * 16)
        out[off], out[off + 4] = _cadd(p, q), _csub(p, q)
        out[off + 2], out[off + 6] = _cadd(m, r), _csub(m, r)
    return out


def _radix8(x0, x1, x2, x3):
    c = np.float32(np.sqrt(0.5))
    a, b = x0 + x2, x0 - x2
    p, q = x1 + x3, x1 - x3
    cp, cq = c * p, c * q
    return ((a + p, a - p), (x0 + cq, -x2 - cp), (b, -q), (x0 - cq, x2 - cp))


def _kernel(u_hbm, are_ref, aim_ref, bre_ref, bim_ref, cre_ref, cim_ref, ldt_ref, dsk_ref,
            eye_ref, m2_hbm, m2i_hbm, ex_hbm, w1_hbm, w2_hbm, w3_hbm, w4_hbm,
            o_hbm,
            u_ref, m2_ref, m2i_ref, ex_ref, w1_v, w2_v, w3_v, w4_v, sems, osems, usems,
            xn_s, h_s, g_s, x3_s, h2_s, o_s, k_s, dt_s, l_s, r_s, z_s, u_s, yx_s, yk_s):
    bf16, f32 = jnp.bfloat16, jnp.float32
    nt = (((1,), (1,)), ((), ()))
    CH = 64

    def u_copy(i):
        rows = pl.ds(i * TM if isinstance(i, int) else pl.multiple_of(i * TM, TM), TM)
        return pltpu.make_async_copy(u_hbm.at[rows, :], u_ref.at[rows, :], usems.at[i])

    copies = [pltpu.make_async_copy(src, dst, sems.at[i]) for i, (src, dst) in enumerate(
        ((w1_hbm, w1_v), (w2_hbm, w2_v), (w3_hbm, w3_v), (w4_hbm, w4_v),
         (ex_hbm, ex_ref), (m2_hbm, m2_ref), (m2i_hbm, m2i_ref)))]
    u_copy(0).start()
    copies[0].start()
    for i in range(1, L // TM):
        u_copy(i).start()

    def fft_pre(src, tb):
        xs = [src[pl.ds(pl.multiple_of(R * (8 * ta) + R * tb, R), R), :] for ta in range(4)]
        for g, (v0, v1) in enumerate(_radix8(*xs)):
            u_s[g, 2 * tb] = v0
            u_s[g, 2 * tb + 1] = v1

    def fft_second(dst, a):
        rows = pl.ds(pl.multiple_of(8 * a, 8), 8)
        for lb in range(D // 128):
            lanes = slice(128 * lb, 128 * (lb + 1))

            def put(k1, v):
                if k1 > 32:
                    k1, v = 64 - k1, (v[0], _scale(v[1], -1.0))
                sl = KORD.index(k1)
                dst[2 * sl, rows, lanes] = v[0]
                dst[2 * sl + 1, rows, lanes] = jnp.zeros_like(v[0]) if v[1] is None else v[1]

            for ka in range(5):
                if ka in (0, 4):
                    t = [(u_s[0, 2 * tb + ka // 4, rows, lanes], None) for tb in range(8)]
                else:
                    t = [(u_s[ka, 2 * tb, rows, lanes], u_s[ka, 2 * tb + 1, rows, lanes]) for tb in range(8)]
                t = [_cconst(t[tb], -tb * ka) for tb in range(8)]
                o = _dft8(t, -1)
                for kb in range(5 if ka == 0 else (4 if ka == 4 else 8)):
                    put(ka + 8 * kb, o[kb])

    def x_stage2(s):
        r0 = pl.multiple_of(s * (2 * R), 2 * R)
        xf = _bdot(m2_ref[pl.ds(r0, 2 * R), :], yx_s[pl.ds(2 * s, 2)].reshape(2 * R, D).astype(bf16))
        yx_s[pl.ds(2 * s, 2)] = xf.reshape(2, R, D)

    def tile(i):
        return pl.ds(i * TM if isinstance(i, int) else pl.multiple_of(i * TM, TM), TM)

    def ln_stage(i):
        xn = _layernorm(u_ref[tile(i), :].astype(f32)).astype(bf16).astype(f32)
        xn_s[tile(i), :] = xn
        x3_s[tile(i), :] = _layernorm(xn).astype(bf16)

    def mix_stage(i):
        r0 = i * TM if isinstance(i, int) else pl.multiple_of(i * TM, TM)
        h_s[pl.ds(PAD + r0, TM), :] = _gelu(_bdot(x3_s[tile(i), :], w1_v[...]))

    def mlp_s1(i):
        r0 = i * TM if isinstance(i, int) else pl.multiple_of(i * TM, TM)
        c = D // 4
        win = h_s[pl.ds(r0 + PAD - 8, TM + 16), :]
        hs = jnp.concatenate([
            win[7:7 + TM, 0 * c:1 * c],
            win[9:9 + TM, 1 * c:2 * c],
            win[6:6 + TM, 2 * c:3 * c],
            win[10:10 + TM, 3 * c:4 * c]], axis=1).astype(bf16)
        x1 = xn_s[tile(i), :] + _bdot(hs, w2_v[...])
        g_s[tile(i), :] = x1
        x3_s[tile(i), :] = _layernorm(x1).astype(bf16)

    def mlp_s2(i):
        for c0 in range(0, FF, HC):
            c1 = min(c0 + HC, FF)
            h2_s[tile(i), c0:c1] = _gelu(jax.lax.dot_general(
                x3_s[tile(i), :], w3_v[c0:c1, :], nt, preferred_element_type=f32)).astype(bf16)
            yield

    def mlp_s3(i):
        for c0 in range(0, D, 128):
            ob = g_s[tile(i), c0:c0 + 128] + _bdot(h2_s[tile(i), :], w4_v[:, c0:c0 + 128])
            g_s[tile(i), c0:c0 + 128] = ob * jax.nn.sigmoid(ob)
            yield

    def run(gen):
        for _ in gen:
            pass

    def one(f, *args):
        f(*args)
        yield

    def interleave(main, side, ratio):
        side = iter(side)
        for _ in main:
            for _ in range(ratio):
                next(side, None)
        for _ in side:
            pass

    def chain(*gens):
        for g in gens:
            yield from g

    def tables(cb, part):
        rows = pl.ds(pl.multiple_of(cb * CH, CH), CH)
        gs = pl.ds(cb * (CH // GC), CH // GC)

        def put_l(i, v):
            l_s[0, gs, i] = v[0].reshape(CH // GC, GC, NS)
            l_s[1, gs, i] = (-v[1]).reshape(CH // GC, GC, NS)

        def get_l(i):
            return l_s[0, gs, i].reshape(CH, NS), -l_s[1, gs, i].reshape(CH, NS)

        def put_r(j, v):
            r_s[0, gs, j] = v[0].reshape(CH // GC, GC, NS)
            r_s[1, gs, j] = v[1].reshape(CH // GC, GC, NS)

        if part == 0:
            z16 = _cexp(16.0 * dt_s[2, rows, :], 16.0 * dt_s[3, rows, :])
            cur = (jnp.ones_like(z16[0]), jnp.zeros_like(z16[0]))
            for j in range(J):
                put_r(j, cur)
                if j + 1 < J:
                    cur = z16 if j == 0 else _cmul(*cur, *z16)
        elif part == 1:
            dtl = dt_s[0, rows, :]
            db_r = dtl * bre_ref[rows, :].astype(f32)
            db_i = dtl * bim_ref[rows, :].astype(f32)
            cur = _cmul(cre_ref[rows, :].astype(f32), cim_ref[rows, :].astype(f32), db_r, db_i)
            z = _cexp(dtl * are_ref[rows, :].astype(f32), dtl * aim_ref[rows, :].astype(f32))
            for b in range(16):
                put_l(b, cur)
                if b + 1 < 16:
                    cur = _cmul(*cur, *z)
            for _ in range(8):
                z = _cmul(*z, *z)
            dt_s[4, rows, :] = z[0]
            dt_s[5, rows, :] = z[1]
        else:
            z256 = (dt_s[4, rows, :], dt_s[5, rows, :])
            lt = {}
            for i in range(16, NI):
                src = BASES[i] - 256
                lt[BASES[i]] = _cmul(*(lt[src] if src in lt else get_l(src)), *z256)
                put_l(i, lt[BASES[i]])

    def block(*work):
        def body(_, c):
            for w in work:
                w()
            return c
        jax.lax.fori_loop(0, 1, body, 0)

    ri = jax.lax.broadcasted_iota(jnp.int32, (NI * GC, J * GC), 0) % GC
    ci = jax.lax.broadcasted_iota(jnp.int32, (NI * GC, J * GC), 1) % GC
    diag = ri + ci == GC - 1

    def kgen_group(g):
        a = jnp.concatenate([l_s[c, g].reshape(NI * GC, NS) for c in range(2)], axis=1).astype(bf16)
        b = jnp.concatenate([r_s[c, g].reshape(J * GC, NS) for c in range(2)], axis=1).astype(bf16)
        o = jax.lax.dot_general(a, b, nt, preferred_element_type=f32)
        o = jnp.where(diag, o, 0.0)
        for hi in range(NH):
            acc = None
            for i in range(8 * hi, min(8 * hi + 8, NI)):
                t = pltpu.roll(o[GC * i:GC * (i + 1), :], 121 - i % 8, 1, stride=1, stride_axis=0)
                acc = t if acc is None else acc + t
            z_s[hi, g] = acc

    with jax.named_scope("phA"):
        for blk in range(D // 128):
            ldt_b = jnp.broadcast_to(ldt_ref[...].reshape(1, D)[:, 128 * blk:128 * (blk + 1)], (NS, 128))
            for rev in range(2):
                dt_s[rev, 128 * blk:128 * (blk + 1), :] = jnp.exp(jax.lax.dot_general(
                    eye_ref[128 * rev:128 * (rev + 1), :], ldt_b, nt,
                    preferred_element_type=f32)).astype(bf16).astype(f32)
            blk_rows = slice(128 * blk, 128 * (blk + 1))
            dt_s[2, blk_rows, :] = dt_s[1, blk_rows, :] * _bdot(eye_ref[128:256, :], are_ref[blk_rows, :])
            dt_s[3, blk_rows, :] = dt_s[1, blk_rows, :] * _bdot(eye_ref[128:256, :], aim_ref[blk_rows, :])
        h_s[0:PAD, :] = jnp.zeros((PAD, D), f32)
        h_s[PAD + L:PAD + L + PAD, :] = jnp.zeros((PAD, D), f32)
        copies[0].wait()

        u_copy(0).wait()
        ln_stage(0)

        def a_body(i, _):
            u_copy(i + 1).wait()
            mix_stage(i)
            ln_stage(i + 1)
            return 0
        jax.lax.fori_loop(0, 2, a_body, 0)
        for c in copies[1:4]:
            c.start()
        jax.lax.fori_loop(2, L // TM - 1, a_body, 0)

    with jax.named_scope("phB"):
        for c in copies[4:]:
            c.start()
        for c in copies[1:4]:
            c.wait()

        P = lambda f, *args: (lambda: run(f(*args)) if f in (mlp_s2, mlp_s3) else f(*args))
        block(P(mix_stage, 7), P(tables, 6, 0), P(tables, 7, 0))
        block(P(mlp_s1, 0), P(tables, 6, 1), P(tables, 7, 1))
        block(P(mlp_s2, 0), P(tables, 6, 2), P(tables, 7, 2))
        block(P(mlp_s1, 1), P(fft_pre, xn_s, 6), P(fft_pre, xn_s, 7))

        def b_body(i, _):
            block(P(mlp_s2, i + 1), P(tables, i, 0), P(tables, i, 1))
            block(P(mlp_s3, i), P(tables, i, 2))
            block(P(mlp_s1, i + 2), P(fft_pre, xn_s, i))
            return 0
        jax.lax.fori_loop(0, 6, b_body, 0)

    with jax.named_scope("phC"):
        def c_body(a, _):
            for q in range(8):
                kgen_group(8 * a + q)
            fft_second(yx_s, a)
            return 0
        jax.lax.fori_loop(0, 8, c_body, 0)

        copies[4].wait()
        copies[5].wait()
        zc = [z_s[hi].reshape(D, 128).astype(bf16) for hi in range(NH)]
        for start, stop, h0 in RANGES:
            if start == 0:
                k_s[start:stop, :] = jax.lax.dot_general(
                    ex_ref[start:stop, :], jnp.concatenate([zc[0], zc[1]], axis=1), nt,
                    preferred_element_type=f32)
            else:
                for r0 in range(start, stop - 8, 256):
                    r1 = min(r0 + 256, stop - 8)
                    k_s[r0:r1, :] = jax.lax.dot_general(
                        ex_ref[r0:r1, 0:128], zc[h0], nt, preferred_element_type=f32)
                k_s[stop - 8:stop, :] = jax.lax.dot_general(
                    ex_ref[stop - 16:stop, :].astype(f32)[8:16].astype(bf16),
                    jnp.concatenate([zc[h0], zc[h0 + 1]], axis=1), nt, preferred_element_type=f32)

    with jax.named_scope("phD"):
        def d1_body(tb, _):
            fft_pre(k_s, tb)
            x_stage2(2 * tb)
            x_stage2(2 * tb + 1)
            return 0
        jax.lax.fori_loop(0, 8, d1_body, 0)

        def d2_body(a, _):
            fft_second(yk_s, a)
            x_stage2(16 + 2 * a)
            x_stage2(17 + 2 * a)
            return 0
        jax.lax.fori_loop(0, 8, d2_body, 0)
        x_stage2(32)

    with jax.named_scope("phE"):
        copies[6].wait()

        def e_body(s, _):
            r0 = pl.multiple_of(s * (2 * R), 2 * R)
            kf = _bdot(m2_ref[pl.ds(r0, 2 * R), :], yk_s[pl.ds(2 * s, 2)].reshape(2 * R, D).astype(bf16))
            pr, pi = _cmul(yx_s[2 * s], yx_s[2 * s + 1], kf[:R], kf[R:])
            p = jnp.concatenate([pr, pi], axis=0).astype(bf16)
            yx_s[pl.ds(2 * s, 2)] = _bdot(m2i_ref[pl.ds(r0, 2 * R), :], p).reshape(2, R, D)
            return 0
        jax.lax.fori_loop(0, NK1, e_body, 0, unroll=11)

    with jax.named_scope("phF"):
        interleave(chain(mlp_s2(7), mlp_s3(6), mlp_s3(7)), [], 0)
        for a in range(8):
            rows = slice(8 * a, 8 * a + 8)
            for lb in range(D // 128):
                lanes = slice(128 * lb, 128 * (lb + 1))

                def get(k1):
                    if k1 > 32:
                        v = get(64 - k1)
                        return v[0], _scale(v[1], -1.0)
                    sl = KORD.index(k1)
                    return (yx_s[2 * sl, rows, lanes],
                            None if k1 in (0, 32) else yx_s[2 * sl + 1, rows, lanes])

                for ka in range(5):
                    o = _dft8([get(ka + 8 * kb) for kb in range(8)], 1)
                    for tb in range(8):
                        if ka in (0, 4):
                            w = _cconst((o[tb][0], None if ka == 0 else o[tb][1]), tb * ka)
                            u_s[0, 2 * tb + ka // 4, rows, lanes] = w[0]
                        else:
                            w = _cconst((_scale(o[tb][0], 2.0), _scale(o[tb][1], 2.0)), tb * ka)
                            u_s[ka, 2 * tb, rows, lanes] = w[0]
                            u_s[ka, 2 * tb + 1, rows, lanes] = w[1]

        dsk = dsk_ref[...].reshape(1, D).astype(f32)

        def out_copy(tb, ta):
            rows = pl.ds(pl.multiple_of(R * (8 * ta) + R * tb, R), R)
            return pltpu.make_async_copy(o_s.at[rows, :], o_hbm.at[rows, :], osems.at[4 * tb + ta])

        def post(tb, _):
            c = np.float32(np.sqrt(0.5))
            w0, w4 = u_s[0, 2 * tb], u_s[0, 2 * tb + 1]
            w1r, w1i = u_s[1, 2 * tb], u_s[1, 2 * tb + 1]
            w2r, w2i = u_s[2, 2 * tb], u_s[2, 2 * tb + 1]
            w3r, w3i = u_s[3, 2 * tb], u_s[3, 2 * tb + 1]
            e, o = w0 + w4, w0 - w4
            p = c * ((w1r - w3r) - (w1i + w3i))
            q = c * ((w3r - w1r) - (w1i + w3i))
            ys = (e + w2r + (w1r + w3r), o - w2i + p, e - w2r + (w3i - w1i), o + w2i + q)
            for ta in range(4):
                rows = pl.ds(pl.multiple_of(R * (8 * ta) + R * tb, R), R)
                s = ys[ta].astype(bf16).astype(f32) + xn_s[rows, :] * dsk
                o_s[rows, :] = (u_ref[rows, :].astype(f32) + s * g_s[rows, :]).astype(bf16)
                out_copy(tb, ta).start()
            return 0
        jax.lax.fori_loop(0, 8, post, 0)
        for tb in range(8):
            for ta in range(4):
                out_copy(tb, ta).wait()


@jax.jit
def pallas_recurrent_scan__ssm_conv_s4__mixer_s_mlp__prompt_kernel(
    A_u: jax.Array,
    A_A_re: jax.Array,
    A_A_im: jax.Array,
    A_B_re: jax.Array,
    A_B_im: jax.Array,
    A_C_re: jax.Array,
    A_C_im: jax.Array,
    A_log_dt: jax.Array,
    A_Dskip: jax.Array,
    B_x: jax.Array,
    B_w1: jax.Array,
    B_w2: jax.Array,
    B_w3: jax.Array,
    B_w4: jax.Array,
):
    m2, m2i, ex, eye = [jnp.asarray(a) for a in _constants()]
    u = A_u.reshape(L, D)
    f32, bf16 = jnp.float32, jnp.bfloat16

    def full(shape):
        return pl.BlockSpec(shape, lambda i: (0,) * len(shape))

    any_spec = pl.BlockSpec(memory_space=pltpu.HBM)
    in_specs = ([any_spec] + [full((D, NS))] * 6 + [full((D,)), full((D,)), full(eye.shape)]
                + [any_spec] * 7)
    scratch = [pltpu.VMEM((L, D), bf16)] + [pltpu.VMEM(c.shape, bf16) for c in (m2, m2i, ex)] + [
        pltpu.VMEM((D, D), bf16), pltpu.VMEM((D, D), bf16),
        pltpu.VMEM((FF, D), bf16), pltpu.VMEM((FF, D), bf16),
        pltpu.SemaphoreType.DMA((7,)), pltpu.SemaphoreType.DMA((32,)), pltpu.SemaphoreType.DMA((L // TM,)),
        pltpu.VMEM((L, D), f32),
        pltpu.VMEM((L + 2 * PAD, D), f32),
        pltpu.VMEM((L, D), f32),
        pltpu.VMEM((L, D), bf16),
        pltpu.VMEM((L, FF), bf16),
        pltpu.VMEM((L, D), bf16),
        pltpu.VMEM((L, D), f32),
        pltpu.VMEM((6, D, NS), f32),
        pltpu.VMEM((2, NG, NI, GC, NS), f32),
        pltpu.VMEM((2, NG, J, GC, NS), f32),
        pltpu.VMEM((NH, NG, GC, J * GC), f32),
        pltpu.VMEM((4, 16, R, D), f32),
        pltpu.VMEM((2 * NK1, R, D), f32),
        pltpu.VMEM((2 * NK1, R, D), f32),
    ]
    out = pl.pallas_call(
        _kernel,
        grid=(1,),
        in_specs=in_specs,
        out_specs=any_spec,
        out_shape=jax.ShapeDtypeStruct((L, D), A_u.dtype),
        scratch_shapes=scratch,
        compiler_params=pltpu.CompilerParams(
            dimension_semantics=("arbitrary",),
            vmem_limit_bytes=127 * 1024 * 1024),
    )(u, A_A_re, A_A_im, A_B_re, A_B_im, A_C_re, A_C_im,
      A_log_dt, A_Dskip, eye, m2, m2i, ex,
      B_w1, B_w2, B_w3.T, B_w4)
    return out.reshape(1, L, D)
```

```python
import jax
import jax.numpy as jnp
import ml_dtypes
import numpy as np
import jax.experimental.pallas as pl
import jax.experimental.pallas.tpu as pltpu

L = 2048
D = 512
NS = 128
FF = 1376
R = 64
NFFT = R * R
NK1 = R // 2 + 1
TM = 256
SLOW_C = -8
SLOW_F = 1
HC = 256
PAD = 16
GC = 8
NG = D // GC
J = 16
BASES = (list(range(16)) + [256 + 2 * m for m in range(8)]
         + [512 + 4 * m for m in range(4)] + [768 + 4 * m for m in range(4)]
         + [1024 + 256 * q + 8 * m for q in range(4) for m in range(2)] + [2048])
NI = len(BASES)
KGROUPS = ([8, 16, 24, 4, 12, 20, 28, 0, 32],
           [1, 9, 17, 25, 7, 15, 23, 31],
           [2, 10, 18, 26, 6, 14, 22, 30],
           [3, 11, 19, 27, 5, 13, 21, 29])
KORD = [k for g in KGROUPS for k in g]
SLOT0 = [0, 9, 17, 25, 33]
RANGES = ((0, 256, 0), (256, 512, 2), (512, 1024, 3), (1024, 2048, 4))
NH = 6


def _lag_table():
    return np.arange(L).astype(ml_dtypes.bfloat16).astype(np.int64)


def _constants():
    bf = ml_dtypes.bfloat16
    t2 = np.arange(R)[None, :]
    k2 = np.arange(R)[:, None]
    m2 = np.zeros((NK1, 2 * R, 2 * R))
    for s, k1 in enumerate(KORD):
        th = -2 * np.pi * ((t2 * (k1 + R * k2)) % NFFT) / NFFT
        cr, ci = np.cos(th), np.sin(th)
        m2[s, :R, :R] = cr
        m2[s, :R, R:] = -ci
        m2[s, R:, :R] = ci
        m2[s, R:, R:] = cr
    m2i = np.transpose(m2, (0, 2, 1)) / NFFT
    lag = _lag_table()
    pos = {b + 16 * j: (i // 8) * 128 + (8 * j - i % 8) % 128 for i, b in enumerate(BASES) for j in range(J)}
    ex = np.zeros((L, 256))
    for start, stop, h0 in RANGES:
        for l in range(start, stop):
            ex[l, pos[int(lag[l])] - 128 * h0] = 1.0
    eye = np.concatenate([np.eye(128), np.kron(np.eye(16), np.eye(8)[::-1])], axis=0)
    return [c.astype(bf) for c in (
        m2.reshape(NK1 * 2 * R, 2 * R), m2i.reshape(NK1 * 2 * R, 2 * R), ex, eye)]


def _layernorm(x):
    m = jnp.mean(x, axis=-1, keepdims=True)
    xc = x - m
    v = jnp.mean(xc * xc, axis=-1, keepdims=True)
    return xc * lax_rsqrt(v + 1e-5)


def lax_rsqrt(v):
    return jax.lax.rsqrt(v)


def _gelu(x):
    c = np.float32(np.sqrt(2.0 / np.pi))
    return 0.5 * x * (1.0 + jnp.tanh(c * (x + 0.044715 * (x * x * x))))


def _cmul(ar, ai, br, bi):
    return ar * br - ai * bi, ar * bi + ai * br


def _cexp(er, ei):
    f = np.float32
    k = jnp.round(ei * f(1.0 / (2.0 * np.pi)))
    r = ((ei - k * f(6.28125)) - k * f(1.9350051879882812e-3)) - k * f(3.0199159819570e-7)
    y = 0.5 * r
    y2 = y * y
    sn = f(-1.0 / 39916800.0)
    for c in (1.0 / 362880.0, -1.0 / 5040.0, 1.0 / 120.0, -1.0 / 6.0, 1.0):
        sn = sn * y2 + f(c)
    sn = sn * y
    cs = f(-1.0 / 87178291200.0)
    for c in (1.0 / 479001600.0, -1.0 / 3628800.0, 1.0 / 40320.0, -1.0 / 720.0, 1.0 / 24.0, -0.5, 1.0):
        cs = cs * y2 + f(c)
    e = jnp.exp(er)
    e2 = e + e
    return e - e2 * (sn * sn), e2 * (sn * cs)


def _bdot(a, b):
    return jnp.dot(a, b, preferred_element_type=jnp.float32)


def _add(a, b):
    return b if a is None else (a if b is None else a + b)


def _sub(a, b):
    return a if b is None else (-b if a is None else a - b)


def _scale(a, c):
    if a is None or c == 0.0:
        return None
    return a if c == 1.0 else (-a if c == -1.0 else np.float32(c) * a)


def _cadd(a, b):
    return _add(a[0], b[0]), _add(a[1], b[1])


def _csub(a, b):
    return _sub(a[0], b[0]), _sub(a[1], b[1])


def _cconst(a, ang):
    ang %= 64
    cr, ci = np.cos(np.pi * ang / 32), np.sin(np.pi * ang / 32)
    if ang % 16 == 0:
        cr, ci = float(round(cr)), float(round(ci))
    return (_sub(_scale(a[0], cr), _scale(a[1], ci)), _add(_scale(a[0], ci), _scale(a[1], cr)))


def _dft8(a, sign):
    s = [_cadd(a[j], a[j + 4]) for j in range(4)]
    d = [_csub(a[j], a[j + 4]) for j in range(4)]
    e = [_cconst(d[j], sign * 8 * j) for j in range(4)]
    out = [None] * 8
    for off, v in ((0, s), (1, e)):
        p, m = _cadd(v[0], v[2]), _csub(v[0], v[2])
        q, r = _cadd(v[1], v[3]), _cconst(_csub(v[1], v[3]), sign * 16)
        out[off], out[off + 4] = _cadd(p, q), _csub(p, q)
        out[off + 2], out[off + 6] = _cadd(m, r), _csub(m, r)
    return out


def _radix8(x0, x1, x2, x3):
    c = np.float32(np.sqrt(0.5))
    a, b = x0 + x2, x0 - x2
    p, q = x1 + x3, x1 - x3
    cp, cq = c * p, c * q
    return ((a + p, a - p), (x0 + cq, -x2 - cp), (b, -q), (x0 - cq, x2 - cp))


def _kernel(u_hbm, are_ref, aim_ref, bre_ref, bim_ref, cre_ref, cim_ref, ldt_ref, dsk_ref,
            eye_ref, m2_hbm, m2i_hbm, ex_hbm, w1_hbm, w2_hbm, w3_hbm, w4_hbm,
            o_hbm,
            u_ref, m2_ref, m2i_ref, ex_ref, w1_v, w2_v, w3_v, w4_v, sems, osems, usems,
            xn_s, h_s, g_s, x3_s, h2_s, o_s, k_s, dt_s, l_s, r_s, z_s, u_s, yx_s, yk_s):
    bf16, f32 = jnp.bfloat16, jnp.float32
    nt = (((1,), (1,)), ((), ()))
    CH = 64

    def u_copy(i):
        rows = pl.ds(i * TM if isinstance(i, int) else pl.multiple_of(i * TM, TM), TM)
        return pltpu.make_async_copy(u_hbm.at[rows, :], u_ref.at[rows, :], usems.at[i])

    copies = [pltpu.make_async_copy(src, dst, sems.at[i]) for i, (src, dst) in enumerate(
        ((w1_hbm, w1_v), (w2_hbm, w2_v), (w3_hbm, w3_v), (w4_hbm, w4_v),
         (ex_hbm, ex_ref), (m2_hbm, m2_ref), (m2i_hbm, m2i_ref)))]
    u_copy(0).start()
    copies[0].start()
    for i in range(1, L // TM):
        u_copy(i).start()

    pace = [None]

    def paced(v):
        return v if pace[0] is None else v + pace[0]

    def paced_b(v):
        if pace[0] is None:
            return v
        t = jnp.concatenate([pace[0]] * (v.shape[1] // 128), axis=1)
        return v + jnp.concatenate([t] * (v.shape[0] // 8), axis=0)

    def set_pace(v, slow=0):
        bits = pltpu.bitcast(v, jnp.int32)
        zero = (bits >> 31) + jax.lax.shift_right_logical(bits, 31)
        for _ in range(slow if slow > 0 else 0):
            zero = pltpu.roll(zero, 1, 1)
        for _ in range(-slow if slow < 0 else 0):
            zero = zero + (zero >> 1)
        pace[0] = zero.astype(f32)

    def fft_pre(src, tb, pacing=False):
        if not pacing:
            xs = [src[pl.ds(pl.multiple_of(R * (8 * ta) + R * tb, R), R), :] for ta in range(4)]
            for g, (v0, v1) in enumerate(_radix8(*xs)):
                u_s[g, 2 * tb] = v0
                u_s[g, 2 * tb + 1] = v1
            return
        for a in range(R // 16):
            xs = [src[pl.ds(pl.multiple_of(R * (8 * ta) + R * tb + 16 * a, 16), 16), :] for ta in range(4)]
            xs[0] = paced_b(xs[0])
            res = _radix8(*xs)
            for g, (v0, v1) in enumerate(res):
                u_s[g, 2 * tb, 16 * a:16 * a + 16, :] = v0
                u_s[g, 2 * tb + 1, 16 * a:16 * a + 16, :] = v1
            set_pace(res[1][1][0:8, 0:128])

    def fft_second(dst, a, pacing=False):
        rows = pl.ds(pl.multiple_of(8 * a, 8), 8)
        for lb in range(D // 128):
            lanes = slice(128 * lb, 128 * (lb + 1))

            def put(k1, v):
                if k1 > 32:
                    k1, v = 64 - k1, (v[0], _scale(v[1], -1.0))
                sl = KORD.index(k1)
                dst[2 * sl, rows, lanes] = v[0]
                dst[2 * sl + 1, rows, lanes] = jnp.zeros_like(v[0]) if v[1] is None else v[1]

            for ka in range(5):
                if ka in (0, 4):
                    t = [(u_s[0, 2 * tb + ka // 4, rows, lanes], None) for tb in range(8)]
                else:
                    t = [(u_s[ka, 2 * tb, rows, lanes], u_s[ka, 2 * tb + 1, rows, lanes]) for tb in range(8)]
                if pacing:
                    t = [(paced(v[0]), v[1]) for v in t]
                t = [_cconst(t[tb], -tb * ka) for tb in range(8)]
                o = _dft8(t, -1)
                for kb in range(5 if ka == 0 else (4 if ka == 4 else 8)):
                    put(ka + 8 * kb, o[kb])
                if pacing:
                    set_pace(o[1][0], SLOW_C)

    def x_stage2(s):
        r0 = pl.multiple_of(s * (2 * R), 2 * R)
        xf = _bdot(m2_ref[pl.ds(r0, 2 * R), :], yx_s[pl.ds(2 * s, 2)].reshape(2 * R, D).astype(bf16))
        yx_s[pl.ds(2 * s, 2)] = xf.reshape(2, R, D)

    def tile(i):
        return pl.ds(i * TM if isinstance(i, int) else pl.multiple_of(i * TM, TM), TM)

    def ln_stage(i):
        xn = _layernorm(u_ref[tile(i), :].astype(f32)).astype(bf16).astype(f32)
        xn_s[tile(i), :] = xn
        x3_s[tile(i), :] = _layernorm(xn).astype(bf16)

    def mix_stage(i):
        r0 = i * TM if isinstance(i, int) else pl.multiple_of(i * TM, TM)
        h_s[pl.ds(PAD + r0, TM), :] = _gelu(_bdot(x3_s[tile(i), :], w1_v[...]))

    def mlp_s1(i):
        r0 = i * TM if isinstance(i, int) else pl.multiple_of(i * TM, TM)
        c = D // 4
        win = h_s[pl.ds(r0 + PAD - 8, TM + 16), :]
        hs = jnp.concatenate([
            win[7:7 + TM, 0 * c:1 * c],
            win[9:9 + TM, 1 * c:2 * c],
            win[6:6 + TM, 2 * c:3 * c],
            win[10:10 + TM, 3 * c:4 * c]], axis=1).astype(bf16)
        x1 = xn_s[tile(i), :] + _bdot(hs, w2_v[...])
        g_s[tile(i), :] = x1
        x3_s[tile(i), :] = _layernorm(x1).astype(bf16)

    def mlp_s2(i):
        for c0 in range(0, FF, HC):
            c1 = min(c0 + HC, FF)
            h2_s[tile(i), c0:c1] = _gelu(jax.lax.dot_general(
                x3_s[tile(i), :], w3_v[c0:c1, :], nt, preferred_element_type=f32)).astype(bf16)
            yield

    def mlp_s3(i):
        for c0 in range(0, D, 128):
            ob = g_s[tile(i), c0:c0 + 128] + _bdot(h2_s[tile(i), :], w4_v[:, c0:c0 + 128])
            g_s[tile(i), c0:c0 + 128] = ob * jax.nn.sigmoid(ob)
            yield

    def run(gen):
        for _ in gen:
            pass

    def one(f, *args):
        f(*args)
        yield

    def interleave(main, side, ratio):
        side = iter(side)
        for _ in main:
            for _ in range(ratio):
                next(side, None)
        for _ in side:
            pass

    def chain(*gens):
        for g in gens:
            yield from g

    def tables(cb, part):
        for q in range(CH // GC):
            tables_group(cb * (CH // GC) + q, part)

    def tables_group(g, part):
        rows = pl.ds(pl.multiple_of(g * GC, GC), GC)

        def put_l(i, v):
            l_s[0, g, i] = v[0]
            l_s[1, g, i] = -v[1]

        def get_l(i):
            return l_s[0, g, i], -l_s[1, g, i]

        def put_r(j, v):
            r_s[0, g, j] = v[0]
            r_s[1, g, j] = v[1]

        if part == 0:
            z16 = _cexp(16.0 * paced(dt_s[2, rows, :]), 16.0 * dt_s[3, rows, :])
            cur = (jnp.ones_like(z16[0]), jnp.zeros_like(z16[0]))
            for j in range(J):
                put_r(j, cur)
                if j + 1 < J:
                    cur = z16 if j == 0 else _cmul(*cur, *z16)
            set_pace(cur[0])
        elif part == 1:
            dtl = paced(dt_s[0, rows, :])
            db_r = dtl * bre_ref[rows, :].astype(f32)
            db_i = dtl * bim_ref[rows, :].astype(f32)
            cur = _cmul(cre_ref[rows, :].astype(f32), cim_ref[rows, :].astype(f32), db_r, db_i)
            z = _cexp(dtl * are_ref[rows, :].astype(f32), dtl * aim_ref[rows, :].astype(f32))
            for b in range(16):
                put_l(b, cur)
                if b + 1 < 16:
                    cur = _cmul(*cur, *z)
            for _ in range(8):
                z = _cmul(*z, *z)
            dt_s[4, rows, :] = z[0]
            dt_s[5, rows, :] = z[1]
            set_pace(z[0] + cur[0])
        else:
            z256 = (paced(dt_s[4, rows, :]), dt_s[5, rows, :])
            lt = {}
            for i in range(16, NI):
                src = BASES[i] - 256
                lt[BASES[i]] = _cmul(*(lt[src] if src in lt else get_l(src)), *z256)
                put_l(i, lt[BASES[i]])
            set_pace(lt[2048][0])

    def block(*work):
        def body(_, c):
            pace[0] = None
            for w in work:
                w()
            pace[0] = None
            return c
        jax.lax.fori_loop(0, 1, body, 0)

    ri = jax.lax.broadcasted_iota(jnp.int32, (NI * GC, J * GC), 0) % GC
    ci = jax.lax.broadcasted_iota(jnp.int32, (NI * GC, J * GC), 1) % GC
    diag = ri + ci == GC - 1

    def kgen_group(g):
        a = jnp.concatenate([l_s[c, g].reshape(NI * GC, NS) for c in range(2)], axis=1).astype(bf16)
        b = jnp.concatenate([r_s[c, g].reshape(J * GC, NS) for c in range(2)], axis=1).astype(bf16)
        o = jax.lax.dot_general(a, b, nt, preferred_element_type=f32)
        o = jnp.where(diag, o, 0.0)
        for hi in range(NH):
            acc = None
            for i in range(8 * hi, min(8 * hi + 8, NI)):
                t = pltpu.roll(o[GC * i:GC * (i + 1), :], 121 - i % 8, 1, stride=1, stride_axis=0)
                acc = t if acc is None else acc + t
            z_s[hi, g] = acc

    with jax.named_scope("phA"):
        for blk in range(D // 128):
            ldt_b = jnp.broadcast_to(ldt_ref[...].reshape(1, D)[:, 128 * blk:128 * (blk + 1)], (NS, 128))
            for rev in range(2):
                dt_s[rev, 128 * blk:128 * (blk + 1), :] = jnp.exp(jax.lax.dot_general(
                    eye_ref[128 * rev:128 * (rev + 1), :], ldt_b, nt,
                    preferred_element_type=f32)).astype(bf16).astype(f32)
            blk_rows = slice(128 * blk, 128 * (blk + 1))
            dt_s[2, blk_rows, :] = dt_s[1, blk_rows, :] * _bdot(eye_ref[128:256, :], are_ref[blk_rows, :])
            dt_s[3, blk_rows, :] = dt_s[1, blk_rows, :] * _bdot(eye_ref[128:256, :], aim_ref[blk_rows, :])
        h_s[0:PAD, :] = jnp.zeros((PAD, D), f32)
        h_s[PAD + L:PAD + L + PAD, :] = jnp.zeros((PAD, D), f32)
        copies[0].wait()

        u_copy(0).wait()
        ln_stage(0)

        def a_body(i, _):
            u_copy(i + 1).wait()
            mix_stage(i)
            ln_stage(i + 1)
            return 0
        jax.lax.fori_loop(0, 2, a_body, 0)
        for c in copies[1:4]:
            c.start()
        jax.lax.fori_loop(2, L // TM - 1, a_body, 0)

    with jax.named_scope("phB"):
        for c in copies[4:]:
            c.start()
        for c in copies[1:4]:
            c.wait()

        P = lambda f, *args: (lambda: run(f(*args)) if f in (mlp_s2, mlp_s3) else f(*args))
        block(P(mix_stage, 7), P(tables, 6, 0), P(tables, 7, 0))
        block(P(mlp_s1, 0), P(tables, 6, 1), P(tables, 7, 1))
        block(P(mlp_s2, 0), P(tables, 6, 2), P(tables, 7, 2))
        block(P(mlp_s1, 1), P(fft_pre, xn_s, 6, True), P(fft_pre, xn_s, 7, True))

        def b_body(i, _):
            block(P(mlp_s2, i + 1), P(tables, i, 1))
            block(P(mlp_s3, i), P(tables, i, 0), P(tables, i, 2))
            block(P(mlp_s1, i + 2), P(fft_pre, xn_s, i, True))
            return 0
        jax.lax.fori_loop(0, 6, b_body, 0)

    with jax.named_scope("phC"):
        def c_body(a, _):
            pace[0] = None
            for q in range(8):
                kgen_group(8 * a + q)
            fft_second(yx_s, a, True)
            pace[0] = None
            return 0
        jax.lax.fori_loop(0, 8, c_body, 0)

        copies[4].wait()
        copies[5].wait()
        zc = [z_s[hi].reshape(D, 128).astype(bf16) for hi in range(NH)]
        for start, stop, h0 in RANGES:
            if start == 0:
                k_s[start:stop, :] = jax.lax.dot_general(
                    ex_ref[start:stop, :], jnp.concatenate([zc[0], zc[1]], axis=1), nt,
                    preferred_element_type=f32)
            else:
                for r0 in range(start, stop - 8, 256):
                    r1 = min(r0 + 256, stop - 8)
                    k_s[r0:r1, :] = jax.lax.dot_general(
                        ex_ref[r0:r1, 0:128], zc[h0], nt, preferred_element_type=f32)
                k_s[stop - 8:stop, :] = jax.lax.dot_general(
                    ex_ref[stop - 16:stop, :].astype(f32)[8:16].astype(bf16),
                    jnp.concatenate([zc[h0], zc[h0 + 1]], axis=1), nt, preferred_element_type=f32)

    with jax.named_scope("phD"):
        def d1_body(tb, _):
            fft_pre(k_s, tb)
            x_stage2(2 * tb)
            x_stage2(2 * tb + 1)
            return 0
        jax.lax.fori_loop(0, 8, d1_body, 0)

        def d2_body(a, _):
            fft_second(yk_s, a)
            x_stage2(16 + 2 * a)
            x_stage2(17 + 2 * a)
            return 0
        jax.lax.fori_loop(0, 8, d2_body, 0)
        x_stage2(32)

    with jax.named_scope("phE"):
        copies[6].wait()

        def e_body(s, _):
            r0 = pl.multiple_of(s * (2 * R), 2 * R)
            kf = _bdot(m2_ref[pl.ds(r0, 2 * R), :], yk_s[pl.ds(2 * s, 2)].reshape(2 * R, D).astype(bf16))
            pr, pi = _cmul(yx_s[2 * s], yx_s[2 * s + 1], kf[:R], kf[R:])
            p = jnp.concatenate([pr, pi], axis=0).astype(bf16)
            yx_s[pl.ds(2 * s, 2)] = _bdot(m2i_ref[pl.ds(r0, 2 * R), :], p).reshape(2, R, D)
            return 0
        jax.lax.fori_loop(0, NK1, e_body, 0, unroll=11)

    with jax.named_scope("phF"):
        def first(a):
            rows = slice(8 * a, 8 * a + 8)
            for lb in range(D // 128):
                lanes = slice(128 * lb, 128 * (lb + 1))

                def get(k1):
                    if k1 > 32:
                        v = get(64 - k1)
                        return v[0], _scale(v[1], -1.0)
                    sl = KORD.index(k1)
                    return (yx_s[2 * sl, rows, lanes],
                            None if k1 in (0, 32) else yx_s[2 * sl + 1, rows, lanes])

                for ka in range(5):
                    o = _dft8([(paced(v[0]), v[1]) for v in [get(ka + 8 * kb) for kb in range(8)]], 1)
                    for tb in range(8):
                        if ka in (0, 4):
                            w = _cconst((o[tb][0], None if ka == 0 else o[tb][1]), tb * ka)
                            u_s[0, 2 * tb + ka // 4, rows, lanes] = w[0]
                        else:
                            w = _cconst((_scale(o[tb][0], 2.0), _scale(o[tb][1], 2.0)), tb * ka)
                            u_s[ka, 2 * tb, rows, lanes] = w[0]
                            u_s[ka, 2 * tb + 1, rows, lanes] = w[1]
                    set_pace(o[1][0], SLOW_F)

        block(P(mlp_s2, 7), P(first, 0), P(first, 1), P(first, 2))
        block(P(mlp_s3, 6), P(first, 3), P(first, 4), P(first, 5))
        block(P(mlp_s3, 7), P(first, 6), P(first, 7))

        dsk = dsk_ref[...].reshape(1, D).astype(f32)

        def out_copy(tb, ta):
            rows = pl.ds(pl.multiple_of(R * (8 * ta) + R * tb, R), R)
            return pltpu.make_async_copy(o_s.at[rows, :], o_hbm.at[rows, :], osems.at[4 * tb + ta])

        def post(tb, _):
            c = np.float32(np.sqrt(0.5))
            w0, w4 = u_s[0, 2 * tb], u_s[0, 2 * tb + 1]
            w1r, w1i = u_s[1, 2 * tb], u_s[1, 2 * tb + 1]
            w2r, w2i = u_s[2, 2 * tb], u_s[2, 2 * tb + 1]
            w3r, w3i = u_s[3, 2 * tb], u_s[3, 2 * tb + 1]
            e, o = w0 + w4, w0 - w4
            p = c * ((w1r - w3r) - (w1i + w3i))
            q = c * ((w3r - w1r) - (w1i + w3i))
            ys = (e + w2r + (w1r + w3r), o - w2i + p, e - w2r + (w3i - w1i), o + w2i + q)
            for ta in range(4):
                rows = pl.ds(pl.multiple_of(R * (8 * ta) + R * tb, R), R)
                s = ys[ta].astype(bf16).astype(f32) + xn_s[rows, :] * dsk
                o_s[rows, :] = (u_ref[rows, :].astype(f32) + s * g_s[rows, :]).astype(bf16)
                out_copy(tb, ta).start()
            return 0
        jax.lax.fori_loop(0, 8, post, 0)
        for tb in range(8):
            for ta in range(4):
                out_copy(tb, ta).wait()


@jax.jit
def pallas_recurrent_scan__ssm_conv_s4__mixer_s_mlp__prompt_kernel(
    A_u: jax.Array,
    A_A_re: jax.Array,
    A_A_im: jax.Array,
    A_B_re: jax.Array,
    A_B_im: jax.Array,
    A_C_re: jax.Array,
    A_C_im: jax.Array,
    A_log_dt: jax.Array,
    A_Dskip: jax.Array,
    B_x: jax.Array,
    B_w1: jax.Array,
    B_w2: jax.Array,
    B_w3: jax.Array,
    B_w4: jax.Array,
):
    m2, m2i, ex, eye = [jnp.asarray(a) for a in _constants()]
    u = A_u.reshape(L, D)
    f32, bf16 = jnp.float32, jnp.bfloat16

    def full(shape):
        return pl.BlockSpec(shape, lambda i: (0,) * len(shape))

    any_spec = pl.BlockSpec(memory_space=pltpu.HBM)
    in_specs = ([any_spec] + [full((D, NS))] * 6 + [full((D,)), full((D,)), full(eye.shape)]
                + [any_spec] * 7)
    scratch = [pltpu.VMEM((L, D), bf16)] + [pltpu.VMEM(c.shape, bf16) for c in (m2, m2i, ex)] + [
        pltpu.VMEM((D, D), bf16), pltpu.VMEM((D, D), bf16),
        pltpu.VMEM((FF, D), bf16), pltpu.VMEM((FF, D), bf16),
        pltpu.SemaphoreType.DMA((7,)), pltpu.SemaphoreType.DMA((32,)), pltpu.SemaphoreType.DMA((L // TM,)),
        pltpu.VMEM((L, D), f32),
        pltpu.VMEM((L + 2 * PAD, D), f32),
        pltpu.VMEM((L, D), f32),
        pltpu.VMEM((L, D), bf16),
        pltpu.VMEM((L, FF), bf16),
        pltpu.VMEM((L, D), bf16),
        pltpu.VMEM((L, D), f32),
        pltpu.VMEM((6, D, NS), f32),
        pltpu.VMEM((2, NG, NI, GC, NS), f32),
        pltpu.VMEM((2, NG, J, GC, NS), f32),
        pltpu.VMEM((NH, NG, GC, J * GC), f32),
        pltpu.VMEM((4, 16, R, D), f32),
        pltpu.VMEM((2 * NK1, R, D), f32),
        pltpu.VMEM((2 * NK1, R, D), f32),
    ]
    out = pl.pallas_call(
        _kernel,
        grid=(1,),
        in_specs=in_specs,
        out_specs=any_spec,
        out_shape=jax.ShapeDtypeStruct((L, D), A_u.dtype),
        scratch_shapes=scratch,
        compiler_params=pltpu.CompilerParams(
            dimension_semantics=("arbitrary",),
            vmem_limit_bytes=127 * 1024 * 1024),
    )(u, A_A_re, A_A_im, A_B_re, A_B_im, A_C_re, A_C_im,
      A_log_dt, A_Dskip, eye, m2, m2i, ex,
      B_w1, B_w2, B_w3.T, B_w4)
    return out.reshape(1, L, D)
```

```python
import jax
import jax.numpy as jnp
import ml_dtypes
import numpy as np
import jax.experimental.pallas as pl
import jax.experimental.pallas.tpu as pltpu

L = 2048
D = 512
NS = 128
FF = 1376
R = 64
NFFT = R * R
NK1 = R // 2 + 1
TM = 256
SLOW_C = -8
SLOW_F = 1
SLOW_E = 1
SLOW_P = 0
NX1 = 3
PACE_D = True
SLOW_K = 1
SLOW_D = 0
HC = 256
PAD = 16
GC = 8
NG = D // GC
J = 16
BASES = (list(range(16)) + [256 + 2 * m for m in range(8)]
         + [512 + 4 * m for m in range(4)] + [768 + 4 * m for m in range(4)]
         + [1024 + 256 * q + 8 * m for q in range(4) for m in range(2)] + [2048])
NI = len(BASES)
KGROUPS = ([8, 16, 24, 4, 12, 20, 28, 0, 32],
           [1, 9, 17, 25, 7, 15, 23, 31],
           [2, 10, 18, 26, 6, 14, 22, 30],
           [3, 11, 19, 27, 5, 13, 21, 29])
KORD = [k for g in KGROUPS for k in g]
SLOT0 = [0, 9, 17, 25, 33]
RANGES = ((0, 256, 0), (256, 512, 2), (512, 1024, 3), (1024, 2048, 4))
NH = 6


def _lag_table():
    return np.arange(L).astype(ml_dtypes.bfloat16).astype(np.int64)


def _constants():
    bf = ml_dtypes.bfloat16
    t2 = np.arange(R)[None, :]
    k2 = np.arange(R)[:, None]
    m2 = np.zeros((NK1, 2 * R, 2 * R))
    for s, k1 in enumerate(KORD):
        th = -2 * np.pi * ((t2 * (k1 + R * k2)) % NFFT) / NFFT
        cr, ci = np.cos(th), np.sin(th)
        m2[s, :R, :R] = cr
        m2[s, :R, R:] = -ci
        m2[s, R:, :R] = ci
        m2[s, R:, R:] = cr
    m2i = np.transpose(m2, (0, 2, 1)) / NFFT
    lag = _lag_table()
    pos = {b + 16 * j: (i // 8) * 128 + (8 * j - i % 8) % 128 for i, b in enumerate(BASES) for j in range(J)}
    ex = np.zeros((L, 256))
    for start, stop, h0 in RANGES:
        for l in range(start, stop):
            ex[l, pos[int(lag[l])] - 128 * h0] = 1.0
    eye = np.concatenate([np.eye(128), np.kron(np.eye(16), np.eye(8)[::-1])], axis=0)
    return [c.astype(bf) for c in (
        m2.reshape(NK1 * 2 * R, 2 * R), m2i.reshape(NK1 * 2 * R, 2 * R), ex, eye)]


def _layernorm(x):
    m = jnp.mean(x, axis=-1, keepdims=True)
    xc = x - m
    v = jnp.mean(xc * xc, axis=-1, keepdims=True)
    return xc * lax_rsqrt(v + 1e-5)


def lax_rsqrt(v):
    return jax.lax.rsqrt(v)


def _gelu(x):
    c = np.float32(np.sqrt(2.0 / np.pi))
    return 0.5 * x * (1.0 + jnp.tanh(c * (x + 0.044715 * (x * x * x))))


def _cmul(ar, ai, br, bi):
    return ar * br - ai * bi, ar * bi + ai * br


def _cexp(er, ei):
    f = np.float32
    k = jnp.round(ei * f(1.0 / (2.0 * np.pi)))
    r = ((ei - k * f(6.28125)) - k * f(1.9350051879882812e-3)) - k * f(3.0199159819570e-7)
    y = 0.5 * r
    y2 = y * y
    sn = f(-1.0 / 39916800.0)
    for c in (1.0 / 362880.0, -1.0 / 5040.0, 1.0 / 120.0, -1.0 / 6.0, 1.0):
        sn = sn * y2 + f(c)
    sn = sn * y
    cs = f(-1.0 / 87178291200.0)
    for c in (1.0 / 479001600.0, -1.0 / 3628800.0, 1.0 / 40320.0, -1.0 / 720.0, 1.0 / 24.0, -0.5, 1.0):
        cs = cs * y2 + f(c)
    e = jnp.exp(er)
    e2 = e + e
    return e - e2 * (sn * sn), e2 * (sn * cs)


def _bdot(a, b):
    return jnp.dot(a, b, preferred_element_type=jnp.float32)


def _add(a, b):
    return b if a is None else (a if b is None else a + b)


def _sub(a, b):
    return a if b is None else (-b if a is None else a - b)


def _scale(a, c):
    if a is None or c == 0.0:
        return None
    return a if c == 1.0 else (-a if c == -1.0 else np.float32(c) * a)


def _cadd(a, b):
    return _add(a[0], b[0]), _add(a[1], b[1])


def _csub(a, b):
    return _sub(a[0], b[0]), _sub(a[1], b[1])


def _cconst(a, ang):
    ang %= 64
    cr, ci = np.cos(np.pi * ang / 32), np.sin(np.pi * ang / 32)
    if ang % 16 == 0:
        cr, ci = float(round(cr)), float(round(ci))
    return (_sub(_scale(a[0], cr), _scale(a[1], ci)), _add(_scale(a[0], ci), _scale(a[1], cr)))


def _dft8(a, sign):
    s = [_cadd(a[j], a[j + 4]) for j in range(4)]
    d = [_csub(a[j], a[j + 4]) for j in range(4)]
    e = [_cconst(d[j], sign * 8 * j) for j in range(4)]
    out = [None] * 8
    for off, v in ((0, s), (1, e)):
        p, m = _cadd(v[0], v[2]), _csub(v[0], v[2])
        q, r = _cadd(v[1], v[3]), _cconst(_csub(v[1], v[3]), sign * 16)
        out[off], out[off + 4] = _cadd(p, q), _csub(p, q)
        out[off + 2], out[off + 6] = _cadd(m, r), _csub(m, r)
    return out


def _radix8(x0, x1, x2, x3):
    c = np.float32(np.sqrt(0.5))
    a, b = x0 + x2, x0 - x2
    p, q = x1 + x3, x1 - x3
    cp, cq = c * p, c * q
    return ((a + p, a - p), (x0 + cq, -x2 - cp), (b, -q), (x0 - cq, x2 - cp))


def _kernel(u_hbm, are_hbm, aim_hbm, bre_hbm, bim_hbm, cre_hbm, cim_hbm, ldt_hbm, dsk_hbm,
            eye_hbm, m2_hbm, m2i_hbm, ex_hbm, w1_hbm, w2_hbm, w3_hbm, w4_hbm,
            o_hbm,
            u_ref, m2_ref, m2i_ref, ex_ref, w1_v, w2_v, w3_v, w4_v, sems, osems, usems,
            xn_s, h_s, g_s, x3_s, h2_s, o_s, k_s, dt_s, l_s, r_s, z_s, u_s, yx_s, yk_s,
            are_ref, aim_ref, bre_ref, bim_ref, cre_ref, cim_ref, ldt_ref, dsk_ref, eye_ref):
    bf16, f32 = jnp.bfloat16, jnp.float32
    nt = (((1,), (1,)), ((), ()))
    CH = 64

    def u_copy(i):
        rows = pl.ds(i * TM if isinstance(i, int) else pl.multiple_of(i * TM, TM), TM)
        return pltpu.make_async_copy(u_hbm.at[rows, :], u_ref.at[rows, :], usems.at[i])

    copies = [pltpu.make_async_copy(src, dst, sems.at[i]) for i, (src, dst) in enumerate(
        ((w1_hbm, w1_v), (w2_hbm, w2_v), (w3_hbm, w3_v), (w4_hbm, w4_v),
         (ex_hbm, ex_ref), (m2_hbm, m2_ref), (m2i_hbm, m2i_ref),
         (are_hbm, are_ref), (aim_hbm, aim_ref), (bre_hbm, bre_ref), (bim_hbm, bim_ref),
         (cre_hbm, cre_ref), (cim_hbm, cim_ref), (ldt_hbm, ldt_ref), (dsk_hbm, dsk_ref),
         (eye_hbm, eye_ref)))]
    u_copy(0).start()
    copies[0].start()
    for i in range(1, L // TM):
        u_copy(i).start()
    for c in copies[7:]:
        c.start()

    pace = [None]

    def paced(v):
        return v if pace[0] is None else v + pace[0]

    def paced_b(v):
        if pace[0] is None:
            return v
        t = jnp.concatenate([pace[0]] * (v.shape[1] // 128), axis=1)
        return v + jnp.concatenate([t] * (v.shape[0] // 8), axis=0)

    def set_pace(v, slow=0):
        bits = pltpu.bitcast(v, jnp.int32)
        zero = (bits >> 31) + jax.lax.shift_right_logical(bits, 31)
        for _ in range(slow if slow > 0 else 0):
            zero = pltpu.roll(zero, 1, 1)
        for _ in range(-slow if slow < 0 else 0):
            zero = zero + (zero >> 1)
        pace[0] = zero.astype(f32)

    def fft_pre(src, tb, pacing=False):
        if not pacing:
            xs = [src[pl.ds(pl.multiple_of(R * (8 * ta) + R * tb, R), R), :] for ta in range(4)]
            for g, (v0, v1) in enumerate(_radix8(*xs)):
                u_s[g, 2 * tb] = v0
                u_s[g, 2 * tb + 1] = v1
            return
        for a in range(R // 16):
            xs = [src[pl.ds(pl.multiple_of(R * (8 * ta) + R * tb + 16 * a, 16), 16), :] for ta in range(4)]
            xs[0] = paced_b(xs[0])
            res = _radix8(*xs)
            for g, (v0, v1) in enumerate(res):
                u_s[g, 2 * tb, 16 * a:16 * a + 16, :] = v0
                u_s[g, 2 * tb + 1, 16 * a:16 * a + 16, :] = v1
            set_pace(res[1][1][0:8, 0:128])

    def fft_second(dst, a, pacing=False, kas=range(5), slow=SLOW_C):
        rows = pl.ds(8 * a if isinstance(a, int) else pl.multiple_of(8 * a, 8), 8)
        for lb in range(D // 128):
            lanes = slice(128 * lb, 128 * (lb + 1))

            def put(k1, v):
                if k1 > 32:
                    k1, v = 64 - k1, (v[0], _scale(v[1], -1.0))
                sl = KORD.index(k1)
                dst[2 * sl, rows, lanes] = v[0]
                dst[2 * sl + 1, rows, lanes] = jnp.zeros_like(v[0]) if v[1] is None else v[1]

            for ka in kas:
                if ka in (0, 4):
                    t = [(u_s[0, 2 * tb + ka // 4, rows, lanes], None) for tb in range(8)]
                else:
                    t = [(u_s[ka, 2 * tb, rows, lanes], u_s[ka, 2 * tb + 1, rows, lanes]) for tb in range(8)]
                if pacing:
                    t = [(paced(v[0]), v[1]) for v in t]
                t = [_cconst(t[tb], -tb * ka) for tb in range(8)]
                o = _dft8(t, -1)
                for kb in range(5 if ka == 0 else (4 if ka == 4 else 8)):
                    put(ka + 8 * kb, o[kb])
                if pacing:
                    set_pace(o[1][0], slow)

    def x_stage2(s):
        r0 = s * (2 * R) if isinstance(s, int) else pl.multiple_of(s * (2 * R), 2 * R)
        xf = _bdot(m2_ref[pl.ds(r0, 2 * R), :], yx_s[pl.ds(2 * s, 2)].reshape(2 * R, D).astype(bf16))
        yx_s[pl.ds(2 * s, 2)] = xf.reshape(2, R, D)

    def tile(i):
        return pl.ds(i * TM if isinstance(i, int) else pl.multiple_of(i * TM, TM), TM)

    def ln_stage(i):
        xn = _layernorm(u_ref[tile(i), :].astype(f32)).astype(bf16).astype(f32)
        xn_s[tile(i), :] = xn
        x3_s[tile(i), :] = _layernorm(xn).astype(bf16)

    def mix_stage(i):
        r0 = i * TM if isinstance(i, int) else pl.multiple_of(i * TM, TM)
        h_s[pl.ds(PAD + r0, TM), :] = _gelu(_bdot(x3_s[tile(i), :], w1_v[...]))

    def mlp_s1(half, q):
        st = isinstance(q, int)
        r0 = (2 * q + half) * TM
        r0 = r0 if st else pl.multiple_of(r0, TM)
        c = D // 4
        win = h_s[pl.ds(r0 + PAD - 8, TM + 16), :]
        hs = jnp.concatenate([
            win[7:7 + TM, 0 * c:1 * c],
            win[9:9 + TM, 1 * c:2 * c],
            win[6:6 + TM, 2 * c:3 * c],
            win[10:10 + TM, 3 * c:4 * c]], axis=1).astype(bf16)
        x1 = xn_s[pl.ds(r0, TM), :] + _bdot(hs, w2_v[...])
        x3 = _layernorm(x1).astype(bf16)
        for m in range(4):
            d0 = TM * (4 * half + m) + R * q
            rows = pl.ds(d0 if st else pl.multiple_of(d0, R), R)
            g_s[rows, :] = x1[R * m:R * (m + 1)]
            x3_s[rows, :] = x3[R * m:R * (m + 1)]

    def mlp_s2(i):
        for c0 in range(0, FF, HC):
            c1 = min(c0 + HC, FF)
            h2_s[tile(i), c0:c1] = _gelu(jax.lax.dot_general(
                x3_s[tile(i), :], w3_v[c0:c1, :], nt, preferred_element_type=f32)).astype(bf16)
            yield

    def mlp_s3(i):
        for c0 in range(0, D, 128):
            ob = g_s[tile(i), c0:c0 + 128] + _bdot(h2_s[tile(i), :], w4_v[:, c0:c0 + 128])
            g_s[tile(i), c0:c0 + 128] = ob * jax.nn.sigmoid(ob)
            yield

    def run(gen):
        for _ in gen:
            pass

    def one(f, *args):
        f(*args)
        yield

    def interleave(main, side, ratio):
        side = iter(side)
        for _ in main:
            for _ in range(ratio):
                next(side, None)
        for _ in side:
            pass

    def chain(*gens):
        for g in gens:
            yield from g

    def tables(cb, part):
        for q in range(CH // GC):
            tables_group(cb * (CH // GC) + q, part)

    def tables_group(g, part):
        rows = pl.ds(pl.multiple_of(g * GC, GC), GC)

        def put_l(i, v):
            l_s[0, g, i] = v[0]
            l_s[1, g, i] = -v[1]

        def get_l(i):
            return l_s[0, g, i], -l_s[1, g, i]

        def put_r(j, v):
            r_s[0, g, j] = v[0]
            r_s[1, g, j] = v[1]

        if part == 0:
            z16 = _cexp(16.0 * paced(dt_s[2, rows, :]), 16.0 * dt_s[3, rows, :])
            cur = (jnp.ones_like(z16[0]), jnp.zeros_like(z16[0]))
            for j in range(J):
                put_r(j, cur)
                if j + 1 < J:
                    cur = z16 if j == 0 else _cmul(*cur, *z16)
            set_pace(cur[0])
        elif part == 1:
            dtl = paced(dt_s[0, rows, :])
            db_r = dtl * bre_ref[rows, :].astype(f32)
            db_i = dtl * bim_ref[rows, :].astype(f32)
            cur = _cmul(cre_ref[rows, :].astype(f32), cim_ref[rows, :].astype(f32), db_r, db_i)
            z = _cexp(dtl * are_ref[rows, :].astype(f32), dtl * aim_ref[rows, :].astype(f32))
            for b in range(16):
                put_l(b, cur)
                if b + 1 < 16:
                    cur = _cmul(*cur, *z)
            for _ in range(8):
                z = _cmul(*z, *z)
            dt_s[4, rows, :] = z[0]
            dt_s[5, rows, :] = z[1]
            set_pace(z[0] + cur[0])
        else:
            z256 = (paced(dt_s[4, rows, :]), dt_s[5, rows, :])
            lt = {}
            for i in range(16, NI):
                src = BASES[i] - 256
                lt[BASES[i]] = _cmul(*(lt[src] if src in lt else get_l(src)), *z256)
                put_l(i, lt[BASES[i]])
            set_pace(lt[2048][0])

    def block(*work):
        def body(_, c):
            pace[0] = None
            for w in work:
                w()
            pace[0] = None
            return c
        jax.lax.fori_loop(0, 1, body, 0)

    ri = jax.lax.broadcasted_iota(jnp.int32, (NI * GC, J * GC), 0) % GC
    ci = jax.lax.broadcasted_iota(jnp.int32, (NI * GC, J * GC), 1) % GC
    diag = ri + ci == GC - 1

    def kgen_group(g):
        a = jnp.concatenate([l_s[c, g].reshape(NI * GC, NS) for c in range(2)], axis=1).astype(bf16)
        b = jnp.concatenate([r_s[c, g].reshape(J * GC, NS) for c in range(2)], axis=1).astype(bf16)
        o = jax.lax.dot_general(a, b, nt, preferred_element_type=f32)
        o = jnp.where(diag, o, 0.0)
        for hi in range(NH):
            acc = None
            for i in range(8 * hi, min(8 * hi + 8, NI)):
                t = pltpu.roll(o[GC * i:GC * (i + 1), :], 121 - i % 8, 1, stride=1, stride_axis=0)
                acc = t if acc is None else acc + t
            z_s[hi, g] = acc

    with jax.named_scope("phA"):
        h_s[0:PAD, :] = jnp.zeros((PAD, D), f32)
        h_s[PAD + L:PAD + L + PAD, :] = jnp.zeros((PAD, D), f32)
        copies[0].wait()

        u_copy(0).wait()
        ln_stage(0)

        def a_body(i, _):
            @pl.when(i == 2)
            def _():
                for c in copies[1:4]:
                    c.start()
            u_copy(i + 1).wait()
            mix_stage(i)
            ln_stage(i + 1)
            return 0
        jax.lax.fori_loop(0, L // TM - 1, a_body, 0)
        for c in copies[7:]:
            c.wait()
        for blk in range(D // 128):
            ldt_b = jnp.broadcast_to(ldt_ref[...].reshape(1, D)[:, 128 * blk:128 * (blk + 1)], (NS, 128))
            for rev in range(2):
                dt_s[rev, 128 * blk:128 * (blk + 1), :] = jnp.exp(jax.lax.dot_general(
                    eye_ref[128 * rev:128 * (rev + 1), :], ldt_b, nt,
                    preferred_element_type=f32)).astype(bf16).astype(f32)
            blk_rows = slice(128 * blk, 128 * (blk + 1))
            dt_s[2, blk_rows, :] = dt_s[1, blk_rows, :] * _bdot(eye_ref[128:256, :], are_ref[blk_rows, :])
            dt_s[3, blk_rows, :] = dt_s[1, blk_rows, :] * _bdot(eye_ref[128:256, :], aim_ref[blk_rows, :])

    with jax.named_scope("phB"):
        for c in copies[4:7]:
            c.start()
        for c in copies[1:4]:
            c.wait()

        P = lambda f, *args: (lambda: run(f(*args)) if f in (mlp_s2, mlp_s3) else f(*args))
        block(P(mix_stage, 7), P(tables, 6, 1))
        block(P(mlp_s1, 0, 0), P(tables, 7, 1), P(tables, 6, 0))
        block(P(mlp_s1, 0, 1), P(tables, 6, 2), P(tables, 7, 0))
        block(P(mlp_s1, 0, 2), P(tables, 7, 2), P(fft_pre, xn_s, 6, True))
        block(P(mlp_s1, 0, 3), P(fft_pre, xn_s, 7, True))
        block(P(mlp_s2, 0), P(tables, 0, 1))

        def b_body(i, _):
            @pl.when(i < 4)
            def _():
                block(P(mlp_s1, 1, i))
            block(P(mlp_s3, i), P(tables, i, 0), P(tables, i, 2))
            block(P(mlp_s2, i + 1), P(tables, jnp.minimum(i + 1, 5), 1), P(fft_pre, xn_s, i, True))
            return 0
        jax.lax.fori_loop(0, 6, b_body, 0)

    with jax.named_scope("phC"):
        def c_body(a, _):
            pace[0] = None
            for q in range(8):
                kgen_group(8 * a + q)
            fft_second(yx_s, a, True)
            pace[0] = None
            return 0
        jax.lax.fori_loop(0, 8, c_body, 0)

        copies[4].wait()
        copies[5].wait()
        zc = [z_s[hi].reshape(D, 128).astype(bf16) for hi in range(NH)]
        for start, stop, h0 in RANGES:
            if start == 0:
                k_s[start:stop, :] = jax.lax.dot_general(
                    ex_ref[start:stop, :], jnp.concatenate([zc[0], zc[1]], axis=1), nt,
                    preferred_element_type=f32)
            else:
                for r0 in range(start, stop - 8, 256):
                    r1 = min(r0 + 256, stop - 8)
                    k_s[r0:r1, :] = jax.lax.dot_general(
                        ex_ref[r0:r1, 0:128], zc[h0], nt, preferred_element_type=f32)
                k_s[stop - 8:stop, :] = jax.lax.dot_general(
                    ex_ref[stop - 16:stop, :].astype(f32)[8:16].astype(bf16),
                    jnp.concatenate([zc[h0], zc[h0 + 1]], axis=1), nt, preferred_element_type=f32)

    with jax.named_scope("phD"):
        def d1_body(h, _):
            pace[0] = None
            for q in range(4 * NX1):
                x_stage2(4 * NX1 * h + q)
            for t in range(4):
                fft_pre(k_s, 4 * h + t, PACE_D)
            pace[0] = None
            return 0
        jax.lax.fori_loop(0, 2, d1_body, 0)

        def x_rest():
            for sl in range(8 * NX1, NK1):
                x_stage2(sl)

        def seconds_k(kas, slow=SLOW_K):
            pace[0] = None
            for a in range(R // 8):
                fft_second(yk_s, a, True, kas, slow)

        block(x_rest, P(seconds_k, (0, 4), SLOW_D))

    def e_slot(s):
        r0 = s * (2 * R) if isinstance(s, int) else pl.multiple_of(s * (2 * R), 2 * R)
        kf = _bdot(m2_ref[pl.ds(r0, 2 * R), :], yk_s[pl.ds(2 * s, 2)].reshape(2 * R, D).astype(bf16))
        pr, pi = _cmul(yx_s[2 * s], yx_s[2 * s + 1], kf[:R], kf[R:])
        p = jnp.concatenate([pr, pi], axis=0).astype(bf16)
        yx_s[pl.ds(2 * s, 2)] = _bdot(m2i_ref[pl.ds(r0, 2 * R), :], p).reshape(2, R, D)

    def first(kas, a, slow):
        rows = slice(8 * a, 8 * a + 8)
        for lb in range(D // 128):
            lanes = slice(128 * lb, 128 * (lb + 1))

            def get(k1):
                if k1 > 32:
                    v = get(64 - k1)
                    return v[0], _scale(v[1], -1.0)
                sl = KORD.index(k1)
                return (yx_s[2 * sl, rows, lanes],
                        None if k1 in (0, 32) else yx_s[2 * sl + 1, rows, lanes])

            for ka in kas:
                o = _dft8([(paced(v[0]), v[1]) for v in [get(ka + 8 * kb) for kb in range(8)]], 1)
                for tb in range(8):
                    if ka in (0, 4):
                        w = _cconst((o[tb][0], None if ka == 0 else o[tb][1]), tb * ka)
                        u_s[0, 2 * tb + ka // 4, rows, lanes] = w[0]
                    else:
                        w = _cconst((_scale(o[tb][0], 2.0), _scale(o[tb][1], 2.0)), tb * ka)
                        u_s[ka, 2 * tb, rows, lanes] = w[0]
                        u_s[ka, 2 * tb + 1, rows, lanes] = w[1]
            set_pace(o[1][0], slow)

    def firsts(kas, slow):
        for a in range(R // 8):
            first(kas, a, slow)

    def e_slots(s0, s1):
        for s in range(s0, s1):
            e_slot(s)

    with jax.named_scope("phE"):
        copies[6].wait()
        def firsts_new(kas):
            pace[0] = None
            firsts(kas, SLOW_E)

        block(P(e_slots, SLOT0[0], SLOT0[1]), P(seconds_k, (1,)))
        block(P(e_slots, SLOT0[1], SLOT0[2]), P(seconds_k, (2,)), P(firsts_new, (0, 4)))
        block(P(e_slots, SLOT0[2], SLOT0[3]), P(seconds_k, (3,)), P(firsts_new, (1,)))
        block(P(e_slots, SLOT0[3], SLOT0[4]), P(firsts_new, (2,)))

    with jax.named_scope("phF"):
        dsk = dsk_ref[...].reshape(1, D).astype(f32)

        def out_copy(tb, ta):
            rows = pl.ds(R * (8 * ta) + R * tb, R)
            return pltpu.make_async_copy(o_s.at[rows, :], o_hbm.at[rows, :], osems.at[4 * tb + ta])

        def post(tb):
            c = np.float32(np.sqrt(0.5))
            for a in range(R // 16):
                rr = slice(16 * a, 16 * a + 16)
                w0, w4 = paced_b(u_s[0, 2 * tb, rr, :]), u_s[0, 2 * tb + 1, rr, :]
                w1r, w1i = u_s[1, 2 * tb, rr, :], u_s[1, 2 * tb + 1, rr, :]
                w2r, w2i = u_s[2, 2 * tb, rr, :], u_s[2, 2 * tb + 1, rr, :]
                w3r, w3i = u_s[3, 2 * tb, rr, :], u_s[3, 2 * tb + 1, rr, :]
                e, o = w0 + w4, w0 - w4
                p = c * ((w1r - w3r) - (w1i + w3i))
                q = c * ((w3r - w1r) - (w1i + w3i))
                ys = (e + w2r + (w1r + w3r), o - w2i + p, e - w2r + (w3i - w1i), o + w2i + q)
                for ta in range(4):
                    r0 = R * (8 * ta) + R * tb + 16 * a
                    rows = slice(r0, r0 + 16)
                    g0 = TM * tb + R * ta + 16 * a
                    s = ys[ta].astype(bf16).astype(f32) + xn_s[rows, :] * dsk
                    res = u_ref[rows, :].astype(f32) + s * g_s[g0:g0 + 16, :]
                    o_s[rows, :] = res.astype(bf16)
                if tb < 7:
                    set_pace(res[0:8, 0:128], SLOW_P)
            for ta in range(4):
                out_copy(tb, ta).start()

        def posts(t0, t1):
            for tb in range(t0, t1):
                post(tb)

        block(P(mlp_s2, 7), P(firsts, (3,), SLOW_F))
        block(P(mlp_s3, 6), P(posts, 0, 4))
        block(P(mlp_s3, 7), P(posts, 4, 7))
        block(P(posts, 7, 8))
        for tb in range(8):
            for ta in range(4):
                out_copy(tb, ta).wait()


@jax.jit
def pallas_recurrent_scan__ssm_conv_s4__mixer_s_mlp__prompt_kernel(
    A_u: jax.Array,
    A_A_re: jax.Array,
    A_A_im: jax.Array,
    A_B_re: jax.Array,
    A_B_im: jax.Array,
    A_C_re: jax.Array,
    A_C_im: jax.Array,
    A_log_dt: jax.Array,
    A_Dskip: jax.Array,
    B_x: jax.Array,
    B_w1: jax.Array,
    B_w2: jax.Array,
    B_w3: jax.Array,
    B_w4: jax.Array,
):
    m2, m2i, ex, eye = [jnp.asarray(a) for a in _constants()]
    u = A_u.reshape(L, D)
    f32, bf16 = jnp.float32, jnp.bfloat16

    def full(shape):
        return pl.BlockSpec(shape, lambda i: (0,) * len(shape))

    any_spec = pl.BlockSpec(memory_space=pltpu.HBM)
    in_specs = ([any_spec] + [any_spec] * 9
                + [any_spec] * 7)
    scratch = [pltpu.VMEM((L, D), bf16)] + [pltpu.VMEM(c.shape, bf16) for c in (m2, m2i, ex)] + [
        pltpu.VMEM((D, D), bf16), pltpu.VMEM((D, D), bf16),
        pltpu.VMEM((FF, D), bf16), pltpu.VMEM((FF, D), bf16),
        pltpu.SemaphoreType.DMA((16,)), pltpu.SemaphoreType.DMA((32,)), pltpu.SemaphoreType.DMA((L // TM,)),
        pltpu.VMEM((L, D), f32),
        pltpu.VMEM((L + 2 * PAD, D), f32),
        pltpu.VMEM((L, D), f32),
        pltpu.VMEM((L, D), bf16),
        pltpu.VMEM((L, FF), bf16),
        pltpu.VMEM((L, D), bf16),
        pltpu.VMEM((L, D), f32),
        pltpu.VMEM((6, D, NS), f32),
        pltpu.VMEM((2, NG, NI, GC, NS), f32),
        pltpu.VMEM((2, NG, J, GC, NS), f32),
        pltpu.VMEM((NH, NG, GC, J * GC), f32),
        pltpu.VMEM((4, 16, R, D), f32),
        pltpu.VMEM((2 * NK1, R, D), f32),
        pltpu.VMEM((2 * NK1, R, D), f32),
    ] + [pltpu.VMEM((D, NS), a.dtype) for a in (A_A_re, A_A_im, A_B_re, A_B_im, A_C_re, A_C_im)] + [
        pltpu.VMEM(a.shape, a.dtype) for a in (A_log_dt, A_Dskip, eye)]
    out = pl.pallas_call(
        _kernel,
        grid=(1,),
        in_specs=in_specs,
        out_specs=any_spec,
        out_shape=jax.ShapeDtypeStruct((L, D), A_u.dtype),
        scratch_shapes=scratch,
        compiler_params=pltpu.CompilerParams(
            dimension_semantics=("arbitrary",),
            vmem_limit_bytes=127 * 1024 * 1024),
    )(u, A_A_re, A_A_im, A_B_re, A_B_im, A_C_re, A_C_im,
      A_log_dt, A_Dskip, eye, m2, m2i, ex,
      B_w1, B_w2, B_w3.T, B_w4)
    return out.reshape(1, L, D)
```
